```python
import os as _os
_os.environ.setdefault("JAX_PLATFORMS", "cpu")
import jax
import jax.numpy as jnp

def _softmax(x, axis=-1):
    return jax.nn.softmax(x, axis=axis)
def _gelu(x):
    return jax.nn.gelu(x, approximate=True)
def _silu(x):
    return jax.nn.silu(x)
def _sigmoid(x):
    return jax.nn.sigmoid(x)
def _layernorm(x, axis=-1, eps=1e-5):
    m = jnp.mean(x, axis=axis, keepdims=True)
    v = jnp.var(x, axis=axis, keepdims=True)
    return (x - m) / jnp.sqrt(v + eps)
def _scatter_add(tgt, idx, src, axis=0):
    return tgt.at[idx].add(src)
def _segment_sum(src, seg, n):
    return jax.ops.segment_sum(src, seg, n)
class _Rng:
    def __init__(self, key):
        self._k = key
    def _next(self):
        self._k, sub = jax.random.split(self._k)
        return sub
    def normal(self, shape):
        return jax.random.normal(self._next(), shape, dtype=jnp.bfloat16)
    def randint(self, lo, hi, shape):
        return jax.random.randint(self._next(), shape, lo, hi, dtype=jnp.int32)
    def uniform(self, shape, lo=0.0, hi=1.0):
        return jax.random.uniform(self._next(), shape, jnp.bfloat16, lo, hi)
    def permutation(self, n):
        return jax.random.permutation(self._next(), n)


kernel_name = 'sequential_preLN__compressed_kv_cla__dense_activation_mish__decode'

def setup_inputs():
    _rng = _Rng(jax.random.key(int.from_bytes(__import__("os").urandom(4), "little")))
    _w = (lambda a: (lambda t: t.astype(jnp.bfloat16) if jnp.issubdtype(t.dtype, jnp.floating) else t)(jnp.asarray(a)))
    def _A_setup():
        B, H, Sq, Sk, D, M = 1, 32, 1, 8192, 128, 512
        Dc = 4 * D
        return {
            "x": _w((lambda *s: _rng.normal(s) * 0.05)(B, Sq, M)),
            "c_kv": _w((lambda *s: _rng.normal(s) * 0.8)(B, Sk, Dc)),
            "w_q": _w((lambda *s: _rng.normal(s) * 0.8)(M, H, D) * (M ** -0.5)),
            "w_uk": _w((lambda *s: _rng.normal(s) * 0.8)(Dc, H, D) * (Dc ** -0.5)),
            "w_uv": _w((lambda *s: _rng.normal(s) * 0.8)(Dc, H, D) * (Dc ** -0.5)),
            "w_o": _w((lambda *s: _rng.normal(s) * 0.8)(H, D, M) * ((H * D) ** -0.5)),
        }
    _A_in = _A_setup()

    def _B_setup():
        B, S, D, F = 1, 1, 512, 1376
        return {
            "x": _w((lambda *s: _rng.normal(s) * 0.05)(B, S, D)),
            "w1": _w((lambda *s: _rng.normal(s) * 0.2)(D, F) * (D ** -0.5)),
            "b1": _w((lambda *s: _rng.normal(s) * 0.05)(F)),
            "w2": _w((lambda *s: _rng.normal(s) * 0.05)(F, D) * (F ** -0.5)),
        }
    _B_in = _B_setup()

    return {
        "A_x": _A_in["x"],
        "A_c_kv": _A_in["c_kv"],
        "A_w_q": _A_in["w_q"],
        "A_w_uk": _A_in["w_uk"],
        "A_w_uv": _A_in["w_uv"],
        "A_w_o": _A_in["w_o"],
        "B_x": _B_in["x"],
        "B_w1": _B_in["w1"],
        "B_b1": _B_in["b1"],
        "B_w2": _B_in["w2"],
    }

def reference(A_x, A_c_kv, A_w_q, A_w_uk, A_w_uv, A_w_o, B_x, B_w1, B_b1, B_w2):
    def _A_ref(x, c_kv, w_q, w_uk, w_uv, w_o):
        B, Sq, M = x.shape[0], x.shape[1], x.shape[2]
        Sk = c_kv.shape[1]
        H, D = w_q.shape[1], w_q.shape[2]
        q = jnp.einsum("bqm,mhd->bhqd", x, w_q)
        k = jnp.einsum("bkc,chd->bhkd", c_kv, w_uk)
        v = jnp.einsum("bkc,chd->bhkd", c_kv, w_uv)
        scores = jnp.einsum("bhqd,bhkd->bhqk", q, k) * (D ** -0.5)
        off = Sk - Sq
        qi = jnp.arange(Sq)[:, None]
        kj = jnp.arange(Sk)[None, :]
        cmask = kj <= (qi + off)
        scores = jnp.where(cmask[None, None], scores, -1e9)
        p = _softmax(scores, axis=-1)
        ctx = jnp.einsum("bhqk,bhkd->bhqd", p, v)
        return jnp.einsum("bhqd,hdm->bqm", ctx, w_o)

    def _B_ref(x, w1, b1, w2):
        h = jnp.einsum("bsd,df->bsf", x, w1) + b1
        sp = jnp.log1p(jnp.exp(-jnp.abs(h))) + jnp.where(h > 0, h, jnp.zeros_like(h))
        act = h * jnp.tanh(sp)
        return jnp.einsum("bsf,fd->bsd", act, w2)

    x = A_x
    h = x + _A_ref(_layernorm(x, axis=-1), A_c_kv, A_w_q, A_w_uk, A_w_uv, A_w_o)
    h2 = h + _B_ref(_layernorm(h, axis=-1), B_w1, B_b1, B_w2)
    return h2
```

```python
import jax
import jax.numpy as jnp
from jax import lax
import jax.experimental.pallas as pl
import jax.experimental.pallas.tpu as pltpu

_F32 = jnp.float32
_BF16 = jnp.bfloat16

_WINDOW = 3
_CH = 128
_KV_CH = 1024
_KV_SUB = 512
_HO = 8
_TG = 8


def _iota(shape, dim):
    return lax.broadcasted_iota(jnp.int32, shape, dim)


def _layernorm(x, eps=1e-5):
    m = jnp.mean(x, axis=-1, keepdims=True)
    xc = x - m
    v = jnp.mean(xc * xc, axis=-1, keepdims=True)
    return xc * lax.rsqrt(v + eps)


def _dot(a, b):
    return jnp.dot(a, b, preferred_element_type=_F32)


def _dot_nt(a, b):
    return lax.dot_general(a, b, (((1,), (1,)), ((), ())), preferred_element_type=_F32)


def _split(total, sizes):
    out, s = [], 0
    for n in sizes:
        out.append((s, n))
        s += n
    assert s == total
    return out


def _ffn_splits(F):
    half = pl.cdiv(pl.cdiv(F, 2), 64) * 64
    f1 = _split(F, (half, F - half)) if F > half else _split(F, (F,))
    a = (F * 15 // 32) // 128 * 128
    b = (F * 12 // 32) // 128 * 128
    sizes = tuple(n for n in (a, b, F - a - b) if n > 0)
    return f1, _split(F, sizes)


def _kernel(x_hbm, ckv_hbm, wq_hbm, wuk_hbm, wuv_hbm, wo_hbm, w1t_hbm, b1_hbm, w2_hbm,
            o_ref,
            x_v, b1_v, ckv_v, wq_v, wuk_v, wuv_v, wo_v, w1t_v, w2_v, sems, ssem):
    M, H, D = wq_v.shape
    Dc = wuk_v.shape[0]
    Sk = ckv_v.shape[0]
    F = w1t_v.shape[0]
    fs1, fs2 = _ffn_splits(F)

    copies, index = [], {}

    def plan(name, src, dst, chunks):
        for i, (s, n) in enumerate(chunks):
            k = len(copies)
            index[(name, i)] = k
            copies.append(pltpu.make_async_copy(
                src.at[pl.ds(s, n)], dst.at[pl.ds(s, n)], sems.at[k % _WINDOW]))

    def even(total, step):
        return [(s, step) for s in range(0, total, step)]

    plan("wq", wq_hbm, wq_v, even(M, _CH))
    plan("wuk", wuk_hbm, wuk_v, even(Dc, _CH))
    plan("ckv", ckv_hbm.at[0], ckv_v, even(Sk, _KV_CH))
    plan("wuv", wuv_hbm, wuv_v, even(Dc, _CH))
    plan("wo", wo_hbm, wo_v, even(H, _HO))
    plan("w1", w1t_hbm, w1t_v, fs1)
    plan("w2", w2_hbm, w2_v, fs2)
    ncopy = len(copies)

    def wait(name, i):
        k = index[(name, i)]
        copies[k].wait()
        if k + _WINDOW < ncopy:
            copies[k + _WINDOW].start()

    x_copy = pltpu.make_async_copy(x_hbm, x_v, ssem.at[0])
    b1_copy = pltpu.make_async_copy(b1_hbm, b1_v, ssem.at[1])
    x_copy.start()
    b1_copy.start()
    for k in range(min(_WINDOW, ncopy)):
        copies[k].start()

    r128 = _iota((128, 128), 0)
    c128 = _iota((128, 128), 1)
    expand = jnp.where((r128 & 3) == (c128 >> 5), 1.0, 0.0).astype(_BF16)
    compact = jnp.where((c128 & 3) == (r128 >> 5), 1.0, 0.0).astype(_BF16)
    r32 = _iota((H, 128), 0)
    c32 = _iota((H, 128), 1)
    head_diag = r32 == (c32 & 31)
    lane_grp = c32 >> 2
    grp_is_row = lane_grp == r32

    x_copy.wait()
    x = x_v[0].astype(_F32)
    xn = _layernorm(x)

    q = jnp.zeros((H, D), _F32)
    for u in range(M // _CH):
        m0 = u * _CH
        xt = jnp.where(grp_is_row, jnp.broadcast_to(xn[:, m0:m0 + 128], (H, 128)), 0.0)
        xr = _dot(xt.astype(_BF16), expand)
        wait("wq", u)
        for g in range(32 // _TG):
            sel = jnp.concatenate(
                [jnp.where(head_diag, jnp.broadcast_to(xr[t:t + 1], (H, 128)), 0.0).astype(_BF16)
                 for t in range(g * _TG, (g + 1) * _TG)], axis=1)
            w = wq_v[pl.ds(m0 + 4 * g * _TG, 4 * _TG)].reshape(4 * _TG * H, D)
            q = q + _dot(sel, w)
    qb = (q * (D ** -0.5)).astype(_BF16)

    qa_tiles = []
    for u in range(Dc // _CH):
        c0 = u * _CH
        wait("wuk", u)
        acc = None
        for g in range(32 // _TG):
            w = wuk_v[pl.ds(c0 + 4 * g * _TG, 4 * _TG)].reshape(4 * _TG * H, D)
            full = _dot_nt(qb, w)
            diag = jnp.concatenate(
                [jnp.where(head_diag, full[:, t * 128:(t + 1) * 128], 0.0).astype(_BF16)
                 for t in range(_TG)], axis=0)
            r = _dot(diag, compact)
            for t in range(_TG):
                blk = r[H * t:H * (t + 1)]
                acc = blk if acc is None else jnp.where(lane_grp == g * _TG + t, blk, acc)
        qa_tiles.append(acc.astype(_BF16))
    qa = jnp.concatenate(qa_tiles, axis=1)

    m_i = jnp.full((H, 1), -jnp.inf, _F32)
    l_i = jnp.zeros((H, 1), _F32)
    acc = jnp.zeros((H, Dc), _F32)
    for u in range(Sk // _KV_CH):
        wait("ckv", u)
        for v in range(_KV_CH // _KV_SUB):
            c = ckv_v[pl.ds(u * _KV_CH + v * _KV_SUB, _KV_SUB), :]
            s = _dot_nt(qa, c)
            m_new = jnp.maximum(m_i, jnp.max(s, axis=-1, keepdims=True))
            alpha = jnp.exp(m_i - m_new)
            p = jnp.exp(s - m_new)
            l_i = alpha * l_i + jnp.sum(p, axis=-1, keepdims=True)
            acc = alpha * acc + _dot(p.astype(_BF16), c)
            m_i = m_new
    cc = acc / l_i

    ctx = jnp.zeros((H, D), _F32)
    for u in range(Dc // _CH):
        c0 = u * _CH
        cu = cc[:, c0:c0 + 128]
        wait("wuv", u)
        for g in range(32 // _TG):
            lhs = jnp.concatenate(
                [jnp.where(lane_grp == g * _TG + t, cu, 0.0).astype(_BF16)
                 for t in range(_TG)], axis=0)
            ex = _dot(lhs, expand)
            sel = jnp.concatenate(
                [jnp.where(head_diag, ex[H * t:H * (t + 1)], 0.0).astype(_BF16)
                 for t in range(_TG)], axis=1)
            w = wuv_v[pl.ds(c0 + 4 * g * _TG, 4 * _TG)].reshape(4 * _TG * H, D)
            ctx = ctx + _dot(sel, w)

    r8 = _iota((8, D), 0)
    out8 = jnp.zeros((8, M), _F32)
    for u in range(H // _HO):
        lhs = jnp.concatenate(
            [jnp.where(r8 == (h % 8), ctx[(h // 8) * 8:(h // 8) * 8 + 8], 0.0).astype(_BF16)
             for h in range(u * _HO, (u + 1) * _HO)], axis=1)
        wait("wo", u)
        out8 = out8 + _dot(lhs, wo_v[pl.ds(u * _HO, _HO)].reshape(_HO * D, M))
    hres = x + jnp.sum(out8, axis=0, keepdims=True)
    hn = _layernorm(hres).astype(_BF16)

    b1_copy.wait()
    b1 = b1_v[...].astype(_F32).reshape(1, F)
    acts = []
    for i, (f0, fn) in enumerate(fs1):
        wait("w1", i)
        h1 = _dot_nt(hn, w1t_v[pl.ds(f0, fn), :]) + b1[:, f0:f0 + fn]
        sp = jnp.log1p(jnp.exp(-jnp.abs(h1))) + jnp.maximum(h1, 0.0)
        acts.append((h1 * jnp.tanh(sp)).astype(_BF16))
    act = jnp.concatenate(acts, axis=1)
    y = hres
    for i, (f0, fn) in enumerate(fs2):
        wait("w2", i)
        y = y + _dot(act[:, f0:f0 + fn], w2_v[pl.ds(f0, fn), :])
    o_ref[0] = y.astype(o_ref.dtype)


@jax.jit
def pallas_sequential_preLN__compressed_kv_cla__dense_activation_mish__decode_kernel(
    A_x: jax.Array,
    A_c_kv: jax.Array,
    A_w_q: jax.Array,
    A_w_uk: jax.Array,
    A_w_uv: jax.Array,
    A_w_o: jax.Array,
    B_x: jax.Array,
    B_w1: jax.Array,
    B_b1: jax.Array,
    B_w2: jax.Array,
):
    del B_x
    B, Sq, M = A_x.shape
    _, Sk, Dc = A_c_kv.shape
    _, H, D = A_w_q.shape
    assert B == 1 and Sq == 1 and H == 32 and D == 128
    assert M % _CH == 0 and Dc % _CH == 0 and Sk % _KV_CH == 0 and H % _HO == 0

    w1t = B_w1.T
    operands = (A_x, A_c_kv, A_w_q, A_w_uk, A_w_uv, A_w_o, w1t, B_b1, B_w2)

    return pl.pallas_call(
        _kernel,
        in_specs=[pl.BlockSpec(memory_space=pl.ANY)] * len(operands),
        out_specs=pl.BlockSpec(memory_space=pltpu.VMEM),
        out_shape=jax.ShapeDtypeStruct(A_x.shape, A_x.dtype),
        scratch_shapes=[
            pltpu.VMEM(A_x.shape, A_x.dtype),
            pltpu.VMEM(B_b1.shape, B_b1.dtype),
            pltpu.VMEM((Sk, Dc), A_c_kv.dtype),
            pltpu.VMEM(A_w_q.shape, A_w_q.dtype),
            pltpu.VMEM(A_w_uk.shape, A_w_uk.dtype),
            pltpu.VMEM(A_w_uv.shape, A_w_uv.dtype),
            pltpu.VMEM(A_w_o.shape, A_w_o.dtype),
            pltpu.VMEM(w1t.shape, w1t.dtype),
            pltpu.VMEM(B_w2.shape, B_w2.dtype),
            pltpu.SemaphoreType.DMA((_WINDOW,)),
            pltpu.SemaphoreType.DMA((2,)),
        ],
        compiler_params=pltpu.CompilerParams(
            vmem_limit_bytes=64 * 1024 * 1024,
            disable_semaphore_checks=True,
            disable_bounds_checks=True,
        ),
    )(*operands)
```
